```python
import os as _os
_os.environ.setdefault("JAX_PLATFORMS", "cpu")
import jax
import jax.numpy as jnp

def _softmax(x, axis=-1):
    return jax.nn.softmax(x, axis=axis)
def _gelu(x):
    return jax.nn.gelu(x, approximate=True)
def _silu(x):
    return jax.nn.silu(x)
def _sigmoid(x):
    return jax.nn.sigmoid(x)
def _layernorm(x, axis=-1, eps=1e-5):
    m = jnp.mean(x, axis=axis, keepdims=True)
    v = jnp.var(x, axis=axis, keepdims=True)
    return (x - m) / jnp.sqrt(v + eps)
def _scatter_add(tgt, idx, src, axis=0):
    return tgt.at[idx].add(src)
def _segment_sum(src, seg, n):
    return jax.ops.segment_sum(src, seg, n)
class _Rng:
    def __init__(self, key):
        self._k = key
    def _next(self):
        self._k, sub = jax.random.split(self._k)
        return sub
    def normal(self, shape):
        return jax.random.normal(self._next(), shape, dtype=jnp.bfloat16)
    def randint(self, lo, hi, shape):
        return jax.random.randint(self._next(), shape, lo, hi, dtype=jnp.int32)
    def uniform(self, shape, lo=0.0, hi=1.0):
        return jax.random.uniform(self._next(), shape, jnp.bfloat16, lo, hi)
    def permutation(self, n):
        return jax.random.permutation(self._next(), n)


kernel_name = 'gated_mix__ssm_conv_h3__ssm_conv_h3__prompt'

def setup_inputs():
    _rng = _Rng(jax.random.key(int.from_bytes(__import__("os").urandom(4), "little")))
    _w = (lambda a: (lambda t: t.astype(jnp.bfloat16) if jnp.issubdtype(t.dtype, jnp.floating) else t)(jnp.asarray(a)))
    def _A_setup():
        B, S, D = 1, 2048, 640
        ks = 4
        return {
            "q": _w((lambda *s: _rng.normal(s) * 0.05)(B, S, D)),
            "k": _w((lambda *s: _rng.normal(s) * 0.05)(B, S, D)),
            "v": _w((lambda *s: _rng.normal(s) * 0.05)(B, S, D)),
            "shift_k": _w((lambda *s: _rng.normal(s) * 0.05)(D, ks) * 0.5),
            "ssm_k": _w((lambda *s: _rng.normal(s) * 0.05)(D, S) * (1.0 / S ** 0.5)),
            "ssm_D": _w((lambda *s: _rng.normal(s) * 0.05)(D)),
        }
    _A_in = _A_setup()

    def _B_setup():
        B, S, D = 1, 2048, 640
        ks = 4
        return {
            "q": _w((lambda *s: _rng.normal(s) * 0.05)(B, S, D)),
            "k": _w((lambda *s: _rng.normal(s) * 0.05)(B, S, D)),
            "v": _w((lambda *s: _rng.normal(s) * 0.05)(B, S, D)),
            "shift_k": _w((lambda *s: _rng.normal(s) * 0.05)(D, ks) * 0.5),
            "ssm_k": _w((lambda *s: _rng.normal(s) * 0.05)(D, S) * (1.0 / S ** 0.5)),
            "ssm_D": _w((lambda *s: _rng.normal(s) * 0.05)(D)),
        }
    _B_in = _B_setup()

    return {
        "A_q": _A_in["q"],
        "A_k": _A_in["k"],
        "A_v": _A_in["v"],
        "A_shift_k": _A_in["shift_k"],
        "A_ssm_k": _A_in["ssm_k"],
        "A_ssm_D": _A_in["ssm_D"],
        "B_q": _B_in["q"],
        "B_k": _B_in["k"],
        "B_v": _B_in["v"],
        "B_shift_k": _B_in["shift_k"],
        "B_ssm_k": _B_in["ssm_k"],
        "B_ssm_D": _B_in["ssm_D"],
        "gate_w": _w((lambda *s: _rng.normal(s) * 0.05)(640) * 16.0),
    }

def reference(A_q, A_k, A_v, A_shift_k, A_ssm_k, A_ssm_D, B_q, B_k, B_v, B_shift_k, B_ssm_k, B_ssm_D, gate_w):
    def _A_ref(q, k, v, shift_k, ssm_k, ssm_D):
        B, S, D = q.shape
        ks = shift_k.shape[-1]
        k_pad = jnp.pad(k, ((0, 0), (ks - 1, 0), (0, 0)))
        k_shift = jnp.zeros_like(k)
        for t in range(ks):
            k_shift = k_shift + k_pad[:, t:t + S, :] * shift_k[:, ks - 1 - t][None, None, :]
        kv = k_shift * v
        L = 2 * S
        kv_pad = jnp.pad(kv, ((0, 0), (0, S), (0, 0)))
        kf_pad = jnp.pad(ssm_k, ((0, 0), (0, S)))
        kv_f = (lambda x, axes=(-2,-1): jnp.fft.rfft2(x.astype(jnp.float32), axes=axes))(kv_pad[:, None, :, :], axes=(1, 2))
        kf_f = (lambda x, axes=(-2,-1): jnp.fft.rfft2(x.astype(jnp.float32), axes=axes))(kf_pad[:, None, :], axes=(1, 2))
        kf_f = (lambda x, *d: x.transpose(*d))(kf_f, 1, 2, 0)
        y_f = kv_f * kf_f[None, :, :, :]
        y = (lambda x, s, axes=(-2,-1): jnp.fft.irfft2(x, s=s, axes=axes).astype(jnp.bfloat16))(y_f, (1, L), axes=(1, 2))[:, 0, :S, :]
        y = y + kv * ssm_D[None, None, :]
        return q * y

    def _B_ref(q, k, v, shift_k, ssm_k, ssm_D):
        B, S, D = q.shape
        ks = shift_k.shape[-1]
        k_pad = jnp.pad(k, ((0, 0), (ks - 1, 0), (0, 0)))
        k_shift = jnp.zeros_like(k)
        for t in range(ks):
            k_shift = k_shift + k_pad[:, t:t + S, :] * shift_k[:, ks - 1 - t][None, None, :]
        kv = k_shift * v
        L = 2 * S
        kv_pad = jnp.pad(kv, ((0, 0), (0, S), (0, 0)))
        kf_pad = jnp.pad(ssm_k, ((0, 0), (0, S)))
        kv_f = (lambda x, axes=(-2,-1): jnp.fft.rfft2(x.astype(jnp.float32), axes=axes))(kv_pad[:, None, :, :], axes=(1, 2))
        kf_f = (lambda x, axes=(-2,-1): jnp.fft.rfft2(x.astype(jnp.float32), axes=axes))(kf_pad[:, None, :], axes=(1, 2))
        kf_f = (lambda x, *d: x.transpose(*d))(kf_f, 1, 2, 0)
        y_f = kv_f * kf_f[None, :, :, :]
        y = (lambda x, s, axes=(-2,-1): jnp.fft.irfft2(x, s=s, axes=axes).astype(jnp.bfloat16))(y_f, (1, L), axes=(1, 2))[:, 0, :S, :]
        y = y + kv * ssm_D[None, None, :]
        return q * y

    x = A_q
    g = _sigmoid((x * gate_w).sum(-1, keepdims=True))
    a = _A_ref(x, A_k, A_v, A_shift_k, A_ssm_k, A_ssm_D)
    b = _B_ref(x, B_k, B_v, B_shift_k, B_ssm_k, B_ssm_D)
    return g * a + (1 - g) * b
```

```python
import numpy as np
import jax
import jax.numpy as jnp
from jax import lax
import jax.experimental.pallas as pl
import jax.experimental.pallas.tpu as pltpu

S = 2048
D = 640
NB = D // 128
def bf16_bits(x):
    u = np.ascontiguousarray(np.asarray(x, np.float32)).view(np.uint32).astype(np.uint64)
    return (((u + 0x7FFF + ((u >> 16) & 1)) >> 16) & 0xFFFF).astype(np.uint32)

def pack_rows(m):
    b = bf16_bits(m)
    return (b[..., 0::2, :] | (b[..., 1::2, :] << 16)).astype(np.uint32)

def make_consts():
    N = 4096
    a = np.arange(32)
    S1 = np.zeros((2, 32, 32))
    S1[0, 0, :] = 1.0
    S1[1, 0, :] = (-1.0) ** a
    for c in range(1, 32):
        S1[0, c, :] = np.cos(2 * np.pi * a * c / 64)
        S1[1, c, :] = -np.sin(2 * np.pi * a * c / 64)
    L1k = np.zeros((128, 64))
    L1h = np.zeros((128, 64))
    jj = np.arange(16)
    for comp in range(2):
        for p in range(2):
            rows = comp * 64 + p * 32 + np.arange(32)
            L1k[np.ix_(rows, 2 * a + p)] = S1[comp]
            for half in range(2):
                aa = 4 * (jj // 2) + (jj % 2) + 2 * half
                L1h[np.ix_(rows, 32 * p + 2 * jj + half)] = S1[comp][:, aa]
    b = np.arange(64)
    e = np.arange(64)
    L2 = np.zeros((32, 128, 128))
    L2i = np.zeros((32, 128, 128))
    for c in range(1, 32):
        T = np.exp(-2j * np.pi * ((b[None, :] * (c + 64 * e[:, None])) % N) / N)
        L2[c, :64, 0::2] = T.real
        L2[c, :64, 1::2] = -T.imag
        L2[c, 64:, 0::2] = T.imag
        L2[c, 64:, 1::2] = T.real
        L2i[c, :64, :64] = T.real.T
        L2i[c, :64, 64:] = T.imag.T
        L2i[c, 64:, :64] = -T.imag.T
        L2i[c, 64:, 64:] = T.real.T
    ep = np.arange(32)
    T0 = np.exp(-2j * np.pi * ((b[None, :] * ep[:, None]) % 64) / 64)
    T32 = np.exp(-2j * np.pi * ((b[None, :] * (32 + 64 * ep[:, None])) % N) / N)
    L2[0, 0:32, 0::2] = T0.real
    L2[0, 64:96, 0::2] = T0.imag
    L2[0, 64, 0::2] = (-1.0) ** b
    L2[0, 32:64, 1::2] = T32.real
    L2[0, 96:128, 1::2] = T32.imag
    w0 = np.full(32, 2.0); w0[0] = 1.0
    L2i[0, :64, 0:32] = (T0.real * w0[:, None]).T
    L2i[0, :64, 64:96] = (T0.imag * w0[:, None]).T
    L2i[0, :64, 64] = (-1.0) ** b
    L2i[0, 64:, 32:64] = 2.0 * T32.real.T
    L2i[0, 64:, 96:128] = 2.0 * T32.imag.T
    S1i = np.zeros((32, 64))
    S1i[:, 0] = 1.0 / N
    S1i[:, 1] = ((-1.0) ** a) / N
    for c in range(1, 32):
        S1i[:, 2 * c] = 2 * np.cos(2 * np.pi * a * c / 64) / N
        S1i[:, 2 * c + 1] = -2 * np.sin(2 * np.pi * a * c / 64) / N
    LF = np.zeros((64, 128))
    for p in range(2):
        LF[p * 32:(p + 1) * 32, p * 64:(p + 1) * 64] = S1i
    return dict(L1h=L1h, L1k=L1k, L2=L2, L2i=L2i, LF=LF)


_M = make_consts()
_t = np.zeros_like(_M['L2i']); _t[:, :, 0::2] = _M['L2i'][:, :, :64]; _t[:, :, 1::2] = _M['L2i'][:, :, 64:]; _M['L2i'] = _t
def _group_rows(m):
    *lead, R2, C = m.shape
    R = R2 // 2
    m = m.reshape(*lead, 2, R // 8, 8, C)
    m = np.moveaxis(m, -4, -3)
    return m.reshape(*lead, R2, C)
_M = {k: _group_rows(v) for k, v in _M.items()}
def _gen_tables():
    k = np.arange(128); b = k // 2; odd = (k % 2 == 1)
    e = np.arange(8)
    F0 = np.exp(-2j * np.pi * ((e[:, None] * b[None, :]) % 64) / 64) * np.where(odd, 1j, 1.0)[None, :]
    w8 = np.exp(-2j * np.pi * (b % 8) / 8)
    s = np.arange(32)
    tw = np.exp(-2j * np.pi * (s[:, None] * b[None, :]) / 4096)
    g = np.zeros((176, 128))
    g[0:8] = F0.real; g[8:16] = F0.imag; g[16] = w8.real; g[17] = w8.imag
    g[24:56] = tw.real; g[56:88] = tw.imag
    col = np.arange(128); bi = 8 * (col // 16) + col % 8; cp = (col // 8) % 2
    row = np.arange(8); ee = row // 2; cc = row % 2
    phi = np.array([[1.0, -1j], [1j, 1.0]])[cp[None, :], cc[:, None]]
    G0 = np.exp(-2j * np.pi * ((ee[:, None] * bi[None, :]) % 64) / 64) * phi
    w4 = np.exp(-2j * np.pi * (bi % 16) / 16)
    twi = np.exp(-2j * np.pi * (s[:, None] * bi[None, :]) / 4096)
    g[88:96] = G0.real; g[96:104] = G0.imag; g[104] = w4.real; g[105] = w4.imag
    g[112:144] = twi.real; g[144:176] = twi.imag
    return g.astype(np.float32)
_GEN = _gen_tables()
_C = {k: pack_rows(np.ascontiguousarray(v)) for k, v in _M.items()}
def _const_blob():
    blob = np.zeros((128 + 32 + 176 + 128, 128), np.uint32)
    blob[0:64, 0:64] = _C['L1h']
    blob[64:128, 0:64] = _C['L1k']
    blob[128:160] = _C['LF']
    blob[160:336] = _GEN.view(np.uint32)
    blob[336:400] = _C['L2'][0]
    blob[400:464] = _C['L2i'][0]
    return blob
_BLOB = _const_blob()
KG = 16
ST1 = 36
ST2 = 68
STH = 68
STK = 36
OFF_Y = 8192
OFF_Z = OFF_Y + 4096
OFF_Q = OFF_Z + 64 * STK
OFF_G = OFF_Q + NB * 1024
AROWS = OFF_G + 2048
NSTEP = NB

f32 = jnp.float32
bf16 = jnp.bfloat16
u32 = jnp.uint32


def _interleave(*lists):
    lists = [list(l) for l in lists if len(l)]
    items = []
    for li, l in enumerate(lists):
        for i, fn in enumerate(l):
            items.append(((i + 0.5) / len(l), li, i, fn))
    items.sort(key=lambda t: (t[0], t[1]))
    for _, _, _, fn in items:
        fn()


def _kernel(aw_hbm, bw_hbm, ad_hbm, bd_hbm, gw_hbm,
            q_hbm, ak_hbm, av_hbm, bk_hbm, bv_hbm, ah_hbm, bh_hbm, c_hbm,
            o_hbm,
            aw_ref, bw_ref, ad_ref, bd_ref, gw_ref, c_ref,
            hbuf, obuf, l2_ref, l2i_ref,
            hpA, hpB, kvA, kvB, t1a, t1b, t1c, t1d, t2A, t2B, arena, prm_ref,
            sem_k, sem_h, sem_q, sem_l, sem_o, sem_s, sem_t):
    j = pl.program_id(0)
    hp_ref = (hpA, hpB); kv_ref = (kvA, kvB); t1_ref = (t1a, t1b, t1c, t1d); t2_ref = (t2A, t2B)
    zero = jnp.minimum(j, 0)
    def aview(off, n):
        return arena.at[pl.ds(pl.multiple_of(zero + off, 8), n)]
    y_ref = (aview(OFF_Y, 2048), aview(OFF_Y + 2048, 2048))
    z_ref = (aview(OFF_Z, 32 * STK), aview(OFF_Z + 32 * STK, 32 * STK))
    g_ref = aview(OFF_G, 2048)
    l1h_w = lambda: pltpu.bitcast(c_ref[0:64, 0:64], bf16)
    l1k_w = lambda: pltpu.bitcast(c_ref[64:128, 0:64], bf16)
    lf_w = lambda: pltpu.bitcast(c_ref[128:160, :], bf16)
    def gen(r0, n):
        return pltpu.bitcast(c_ref[160 + r0:160 + r0 + n, :], f32)
    blk_of = lambda t: t
    jd = blk_of(j)
    jq = blk_of(jnp.maximum(j - 1, 0))
    slot = j % 2

    def unpack(x):
        e = pltpu.unpack_elementwise(x, index=0, packed_dtype=bf16, unpacked_dtype=f32)
        o = pltpu.unpack_elementwise(x, index=1, packed_dtype=bf16, unpacked_dtype=f32)
        return e, o

    def pack(lo, hi):
        return pltpu.pack_elementwise([lo, hi], packed_dtype=bf16)

    def asbf(x):
        return pltpu.bitcast(x, bf16)

    kv_hbm = (ak_hbm, av_hbm, bk_hbm, bv_hbm)
    h_hbm = (ah_hbm, bh_hbm)

    def cols(blk):
        return pl.ds(blk * 128, 128) if isinstance(blk, int) else pl.ds(pl.multiple_of(blk * 128, 128), 128)

    def kview(sl, i):
        return aview(sl * 4096 + i * 1024, 1024)

    def qview(blk):
        return aview(OFF_Q + blk * 1024, 1024)

    def k_copy(blk, sl, i):
        return pltpu.make_async_copy(kv_hbm[i].at[:, cols(blk)], kview(sl, i).bitcast(bf16), sem_k.at[sl, i])

    def h_copy(blk, sl, i):
        return pltpu.make_async_copy(h_hbm[i].at[cols(blk), :], hbuf.at[sl, i], sem_h.at[sl, i])

    def q_copy(i):
        return pltpu.make_async_copy(q_hbm.at[:, cols(i)], qview(i).bitcast(bf16), sem_q.at[i])

    def c_copy():
        return pltpu.make_async_copy(c_hbm, c_ref, sem_l.at[0])

    def o_copy(blk, sl):
        return pltpu.make_async_copy(obuf.at[sl], o_hbm.at[:, cols(blk)], sem_o.at[sl])

    def start_block(blk, sl):
        h_copy(blk, sl, 0).start()
        h_copy(blk, sl, 1).start()
        for i in range(4):
            k_copy(blk, sl, i).start()

    def waits(*cs):
        def f():
            for c in cs:
                c.wait()
        return f

    row8 = jax.lax.broadcasted_iota(jnp.int32, (8, 128), 0)
    row64 = jax.lax.broadcasted_iota(jnp.int32, (64, 128), 0)
    L = lambda r: asbf(r[...])
    WS = lambda br: tuple(prm_ref[jd, pl.ds(4 * br + i, 1), :] for i in range(4))
    DD = lambda br: prm_ref[jd, pl.ds(8 + br, 1), :]

    def pk(r, g, c0=0):
        return pack(r[16 * g:16 * g + 8, c0:c0 + 128], r[16 * g + 8:16 * g + 16, c0:c0 + 128])

    def store_t1(ref, r, be):
        for g in range(8):
            ref[pl.ds((2 * be + g // 4) * ST1 + 8 * (g % 4), 8), :] = pk(r, g)

    def hprep(br):
        def item(tau):
            def f():
                h_ref = hbuf.at[slot, br]
                x0 = h_ref[:, pl.ds(256 * tau, 128)].astype(f32)
                x1 = h_ref[:, pl.ds(256 * tau + 128, 128)].astype(f32)
                w = pack(x0, x1).T
                hp_ref[br][pl.ds((2 * tau) * STH, 64), :] = w[:64]
                hp_ref[br][pl.ds((2 * tau + 1) * STH, 64), :] = w[64:]
            return f
        return [item(t) for t in range(8)]

    def hstage(br):
        def item(be):
            def f():
                x = jnp.concatenate([hp_ref[br][pl.ds(2 * be + p, 16, stride=STH), :] for p in range(2)], axis=0)
                r = jnp.dot(l1h_w(), asbf(x), preferred_element_type=f32)
                store_t1(t1_ref[2 * br], r, be)
            return f
        return [item(be) for be in range(32)]

    def kprep(br, blk, sl):
        wc = []
        def item(m0):
            def f():
                if not wc:
                    wc.append(tuple(prm_ref[blk, pl.ds(4 * br + i, 1), :] for i in range(4)))
                w0, w1, w2, w3 = wc[0]
                ku = kview(sl, 2 * br)
                vu = kview(sl, 2 * br + 1)
                c = ku[pl.ds(m0, KG), :]
                if m0 == 0:
                    f8 = ku[pl.ds(0, 8), :]
                    p1 = jnp.where(row8 < 1, jnp.uint32(0), pltpu.roll(f8, 1, 0))
                    p2 = jnp.where(row8 < 2, jnp.uint32(0), pltpu.roll(f8, 2, 0))
                    if KG > 8:
                        p1 = jnp.concatenate([p1, ku[pl.ds(7, KG - 8), :]], axis=0)
                        p2 = jnp.concatenate([p2, ku[pl.ds(6, KG - 8), :]], axis=0)
                else:
                    p1 = ku[pl.ds(m0 - 1, KG), :]
                    p2 = ku[pl.ds(m0 - 2, KG), :]
                e, o = unpack(c)
                e1, o1 = unpack(p1)
                o2 = pltpu.unpack_elementwise(p2, index=1, packed_dtype=bf16, unpacked_dtype=f32)
                ve, vo = unpack(vu[pl.ds(m0, KG), :])
                kse = w0 * e + w1 * o1 + w2 * e1 + w3 * o2
                kso = w0 * o + w1 * e + w2 * o1 + w3 * e1
                kv_ref[br][pl.ds((m0 // 32) * STK + m0 % 32, KG), :] = pack(kse * ve, kso * vo)
            return f
        return [item(m0) for m0 in range(0, 1024, KG)]

    def kstage(br):
        def item(be):
            def f():
                x = kv_ref[br][pl.ds(be, 32, stride=STK), :]
                r = jnp.dot(l1k_w(), asbf(x), preferred_element_type=f32)
                store_t1(t1_ref[2 * br + 1], r, be)
            return f
        return [item(be) for be in range(32)]

    def s2(br, side=None):
        def item(s):
            def f():
                x = jnp.concatenate([t1_ref[2 * br + i][pl.ds(s, 64, stride=ST1), :] for i in range(2)], axis=1)
                zz = jnp.dot(asbf(l2_ref.at[s].bitcast(u32)[...]), asbf(x), preferred_element_type=f32)
                ddv = DD(br)
                for g in range(8):
                    gr = zz[16 * g:16 * g + 8, :128] + ddv
                    gi = zz[16 * g + 8:16 * g + 16, :128]
                    zr = zz[16 * g:16 * g + 8, 128:]
                    zi = zz[16 * g + 8:16 * g + 16, 128:]
                    if s == 0 and g == 0:
                        gi = jnp.where(row8 == 0, gi + ddv, gi)
                        yr = jnp.where(row8 == 0, zr * gr, zr * gr - zi * gi)
                        yi = jnp.where(row8 == 0, zi * gi, zr * gi + zi * gr)
                    else:
                        yr = zr * gr - zi * gi
                        yi = zr * gi + zi * gr
                    y_ref[br][pl.ds(s * 64 + 8 * g, 8), :] = pack(yr, yi)
                    if side is not None:
                        side(s * 8 + g)
            return f
        return [item(s) for s in range(32)]

    def paced(total, *lists):
        pos = [0] * len(lists)
        def side(n):
            for li, l in enumerate(lists):
                due = ((n + 1) * len(l)) // total
                while pos[li] < due:
                    l[pos[li]]()
                    pos[li] += 1
        return side

    def s2i(side=None):
        def item(s):
            def f():
                y = jnp.concatenate([y_ref[br][pl.ds(s * 64, 64), :] for br in range(2)], axis=1)
                u = jnp.dot(asbf(l2i_ref.at[s].bitcast(u32)[...]), asbf(y), preferred_element_type=f32)
                for g in range(8):
                    for br in range(2):
                        t2_ref[br][pl.ds(s * ST2 + 8 * g, 8), :] = pk(u, g, 128 * br)
                        if side is not None:
                            side(s * 16 + g * 2 + br)
            return f
        return [item(s) for s in range(32)]

    def fin():
        def item(be):
            def f():
                x = jnp.concatenate(
                    [jnp.concatenate([t2_ref[i][pl.ds(2 * be + p, 32, stride=ST2), :] for i in range(2)], axis=1)
                     for p in range(2)], axis=0)
                y = jnp.dot(lf_w(), asbf(x), preferred_element_type=f32)
                for g in range(4):
                    for br in range(2):
                        z_ref[br][pl.ds(8 * g * STK + be, 8, stride=STK), :] = pk(y, g, 128 * br)
            return f
        return [item(be) for be in range(32)]

    def epi(qoff, osl):
        def item(m0):
            def f():
                qu = aview(qoff, 1024)
                ou = obuf.at[osl].bitcast(u32)
                zrow = (m0 // 32) * STK + m0 % 32
                ae, ao = unpack(z_ref[0][pl.ds(zrow, KG), :])
                be_, bo = unpack(z_ref[1][pl.ds(zrow, KG), :])
                ge = pltpu.bitcast(g_ref[pl.ds(2 * m0, KG, stride=2), :], f32)
                go = pltpu.bitcast(g_ref[pl.ds(2 * m0 + 1, KG, stride=2), :], f32)
                qe, qo = unpack(qu[pl.ds(m0, KG), :])
                ou[pl.ds(m0, KG), :] = pack(qe * (be_ + ge * (ae - be_)), qo * (bo + go * (ao - bo)))
            return f
        return [item(m0) for m0 in range(0, 1024, KG)]

    def cmul(ar, ai, br_, bi_):
        return ar * br_ - ai * bi_, ar * bi_ + ai * br_

    def gen_fwd(slist):
        f0u, f0v = gen(0, 8), gen(8, 8)
        w8r, w8i = gen(16, 1), gen(17, 1)
        for s in slist:
            U, V = cmul(f0u, f0v, gen(24 + s, 1), gen(56 + s, 1))
            blocks = []
            for g in range(8):
                blocks += [U, V]
                if g < 7:
                    U, V = cmul(U, V, w8r, w8i)
            l2_ref[s] = jnp.concatenate(blocks, axis=0).astype(bf16)

    def gen_inv(slist):
        g0r, g0i = gen(88, 8), gen(96, 8)
        w4r, w4i = gen(104, 1), gen(105, 1)
        for s in slist:
            U, V = cmul(g0r, g0i, gen(112 + s, 1), gen(144 + s, 1))
            blocks = []
            for v in range(16):
                blocks.append(U)
                if v < 15:
                    U, V = cmul(U, V, w4r, w4i)
            l2i_ref[s] = jnp.concatenate(blocks, axis=0).T.astype(bf16)

    def gate():
        for i in range(NB):
            q_copy(i).wait()
        w = gw_ref[...].reshape(1, D)
        for c in range(4):
            z = None
            for jb in range(NB):
                w16 = jnp.broadcast_to(w[:, jb * 128:(jb + 1) * 128], (16, 128))
                qq = asbf(qview(jb)[pl.ds(c * 256, 256), :])
                t = lax.dot_general(w16, qq, (((1,), (1,)), ((), ())), preferred_element_type=f32)
                z = t if z is None else z + t
            g = 0.5 * jnp.tanh(0.5 * z[:8]) + 0.5
            for t in range(4):
                gt = jnp.broadcast_to(g[0:1, t * 128:(t + 1) * 128], (128, 128))
                g_ref[pl.ds((4 * c + t) * 128, 128), :] = pltpu.bitcast(gt.T, u32)

    osl = (j + 1) % 2

    def run(items):
        for it in items:
            it()

    small = ((aw_hbm, aw_ref), (bw_hbm, bw_ref), (ad_hbm, ad_ref), (bd_hbm, bd_ref), (gw_hbm, gw_ref))
    def s_copy(i):
        return pltpu.make_async_copy(small[i][0], small[i][1], sem_s.at[i])

    def start_k(blk, sl):
        for i in range(4):
            k_copy(blk, sl, i).start()

    def start_h(blk, sl):
        for i in range(2):
            h_copy(blk, sl, i).start()

    def wait_k(sl, idx=(0, 1, 2, 3)):
        for i in idx:
            k_copy(0, sl, i).wait()


    @pl.when(j == 0)
    def _first():
        c_copy().start()
        h_copy(0, 0, 0).start()
        g_ref[...] = jnp.zeros((2048, 128), u32)
        c_copy().wait()
        for i in range(len(small)):
            s_copy(i).start()
        k_copy(0, 0, 0).start()
        k_copy(0, 0, 1).start()
        l2_ref[0] = pltpu.bitcast(c_ref[336:400, :], bf16)
        l2i_ref[0] = pltpu.bitcast(c_ref[400:464, :], bf16)
        gen_fwd(range(1, 32))
        h_copy(0, 0, 0).wait()
        h_copy(0, 0, 1).start()
        run(hprep(0))
        _interleave(hstage(0), [lambda s=s: gen_inv([s]) for s in range(1, 20)])
        for i in range(len(small)):
            s_copy(i).wait()
        wait_k(0, (0, 1))
        k_copy(0, 0, 2).start()
        k_copy(0, 0, 3).start()
        adv = ad_ref[...].astype(f32).reshape(1, D)
        bdv = bd_ref[...].astype(f32).reshape(1, D)
        awv = aw_ref[...].astype(f32)
        bwv = bw_ref[...].astype(f32)
        for i in range(NB):
            c0 = i * 128
            prm_ref[i] = jnp.concatenate(
                [awv[:, c0:c0 + 128], bwv[:, c0:c0 + 128], adv[:, c0:c0 + 128], bdv[:, c0:c0 + 128],
                 jnp.zeros((6, 128), f32)], axis=0)
        run(kprep(0, 0, 0))
        h_copy(0, 0, 1).wait()
        start_k(1, 1)
        _interleave(kstage(0), hprep(1))
        gi = [lambda s=s: gen_inv([s]) for s in range(20, 32)]
        _interleave(s2(0), gi)
        wait_k(0, (2, 3))
        start_h(1, 1)
        _interleave(hstage(1), kprep(1, 0, 0))
        run(kstage(1))
        wait_k(1, (0, 1))
        run(s2(1, paced(256, kprep(0, 1, 1))))
        wait_k(1, (2, 3))
        start_k(blk_of(2), 0)
        _interleave(s2i(), kprep(1, 1, 1))

    osl = (j + 1) % 2
    nxt = blk_of(jnp.minimum(j + 1, NSTEP - 1))

    @pl.when(j > 0)
    def _steady():
        more = j + 1 < NSTEP
        h_copy(0, slot, 0).wait()
        h_copy(0, slot, 1).wait()
        @pl.when(j == 1)
        def _():
            for i in range(NB):
                q_copy(i).start()
        pl.when(more)(lambda: start_h(nxt, 1 - slot))
        pl.when(j >= 3)(waits(o_copy(0, osl)))
        _interleave(fin(), hprep(0))
        _interleave(hstage(0), hprep(1))
        run(hstage(1))
        run(kstage(0))
        run(kstage(1))
        pl.when(more)(lambda: wait_k(1 - slot))
        pl.when(j + 2 < NSTEP)(lambda: start_k(blk_of(j + 2), slot))
        ep = epi(jnp.where(j == 1, OFF_G, OFF_Q + jq * 1024), osl)
        run(s2(0, paced(256, kprep(0, nxt, 1 - slot), ep[:len(ep) // 2])))
        run(s2(1, paced(256, kprep(1, nxt, 1 - slot), ep[len(ep) // 2:])))
        run(s2i())
        @pl.when(j == 1)
        def _():
            gate()
            run(epi(OFF_Q + jq * 1024, osl))
        o_copy(jq, osl).start()

    @pl.when(j == NSTEP - 1)
    def _():
        osl2 = j % 2
        run(fin())
        o_copy(0, osl2).wait()
        ep2 = epi(OFF_Q + jd * 1024, osl2)
        NC = 8
        n = len(ep2) // NC
        cps = []
        for c in range(NC):
            run(ep2[c * n:(c + 1) * n])
            rows = pl.ds(c * (S // NC), S // NC)
            cp = pltpu.make_async_copy(obuf.at[osl2, rows, :], o_hbm.at[rows, cols(jd)], sem_t.at[c])
            cp.start()
            cps.append(cp)
        o_copy(0, osl).wait()
        for cp in cps:
            cp.wait()


@jax.jit
def pallas_gated_mix__ssm_conv_h3__ssm_conv_h3__prompt_kernel(A_q, A_k, A_v, A_shift_k, A_ssm_k, A_ssm_D, B_q, B_k, B_v, B_shift_k, B_ssm_k, B_ssm_D, gate_w):
    q = A_q.reshape(S, D)
    ak = A_k.reshape(S, D); av = A_v.reshape(S, D)
    bk = B_k.reshape(S, D); bv = B_v.reshape(S, D)
    aw = A_shift_k.T
    bw = B_shift_k.T
    vm = pl.BlockSpec(memory_space=pltpu.VMEM)
    anyspec = pl.BlockSpec(memory_space=pl.ANY)
    out = pl.pallas_call(
        _kernel,
        grid=(NSTEP,),
        in_specs=[anyspec] * 13,
        out_specs=anyspec,
        out_shape=jax.ShapeDtypeStruct((S, D), jnp.bfloat16),
        scratch_shapes=[
            pltpu.VMEM((4, D), bf16), pltpu.VMEM((4, D), bf16),
            pltpu.VMEM((D,), bf16), pltpu.VMEM((D,), bf16), pltpu.VMEM((D,), bf16),
            pltpu.VMEM(_BLOB.shape, u32),
            pltpu.VMEM((2, 2, 128, S), bf16),
            pltpu.VMEM((2, S, 128), bf16),
            pltpu.VMEM((32, 128, 128), bf16),
            pltpu.VMEM((32, 128, 128), bf16),
            *[pltpu.VMEM((16 * STH, 128), u32)] * 2,
            *[pltpu.VMEM((32 * STK, 128), u32)] * 2,
            *[pltpu.VMEM((64 * ST1, 128), u32)] * 4,
            *[pltpu.VMEM((32 * ST2, 128), u32)] * 2,
            pltpu.VMEM((AROWS, 128), u32),
            pltpu.VMEM((NB, 16, 128), f32),
            pltpu.SemaphoreType.DMA((2, 4)),
            pltpu.SemaphoreType.DMA((2, 2)),
            pltpu.SemaphoreType.DMA((NB,)),
            pltpu.SemaphoreType.DMA((1,)),
            pltpu.SemaphoreType.DMA((2,)),
            pltpu.SemaphoreType.DMA((5,)),
            pltpu.SemaphoreType.DMA((8,)),
        ],
        compiler_params=pltpu.CompilerParams(
            dimension_semantics=("arbitrary",), vmem_limit_bytes=100 * 1024 * 1024),
    )(aw, bw, A_ssm_D, B_ssm_D, gate_w,
      q, ak, av, bk, bv, A_ssm_k, B_ssm_k, jnp.asarray(_BLOB))
    return out.reshape(1, S, D)
```

```python
import numpy as np
import jax
import jax.numpy as jnp
from jax import lax
import jax.experimental.pallas as pl
import jax.experimental.pallas.tpu as pltpu

S = 2048
D = 640
NB = D // 128
def bf16_bits(x):
    u = np.ascontiguousarray(np.asarray(x, np.float32)).view(np.uint32).astype(np.uint64)
    return (((u + 0x7FFF + ((u >> 16) & 1)) >> 16) & 0xFFFF).astype(np.uint32)

def pack_rows(m):
    b = bf16_bits(m)
    return (b[..., 0::2, :] | (b[..., 1::2, :] << 16)).astype(np.uint32)

def make_consts():
    N = 4096
    a = np.arange(32)
    S1 = np.zeros((2, 32, 32))
    S1[0, 0, :] = 1.0
    S1[1, 0, :] = (-1.0) ** a
    for c in range(1, 32):
        S1[0, c, :] = np.cos(2 * np.pi * a * c / 64)
        S1[1, c, :] = -np.sin(2 * np.pi * a * c / 64)
    L1k = np.zeros((128, 64))
    L1h = np.zeros((128, 64))
    jj = np.arange(16)
    for comp in range(2):
        for p in range(2):
            rows = comp * 64 + p * 32 + np.arange(32)
            L1k[np.ix_(rows, 2 * a + p)] = S1[comp]
            for half in range(2):
                aa = 4 * (jj // 2) + (jj % 2) + 2 * half
                L1h[np.ix_(rows, 32 * p + 2 * jj + half)] = S1[comp][:, aa]
    b = np.arange(64)
    e = np.arange(64)
    L2 = np.zeros((32, 128, 128))
    L2i = np.zeros((32, 128, 128))
    for c in range(1, 32):
        T = np.exp(-2j * np.pi * ((b[None, :] * (c + 64 * e[:, None])) % N) / N)
        L2[c, :64, 0::2] = T.real
        L2[c, :64, 1::2] = -T.imag
        L2[c, 64:, 0::2] = T.imag
        L2[c, 64:, 1::2] = T.real
        L2i[c, :64, :64] = T.real.T
        L2i[c, :64, 64:] = T.imag.T
        L2i[c, 64:, :64] = -T.imag.T
        L2i[c, 64:, 64:] = T.real.T
    ep = np.arange(32)
    T0 = np.exp(-2j * np.pi * ((b[None, :] * ep[:, None]) % 64) / 64)
    T32 = np.exp(-2j * np.pi * ((b[None, :] * (32 + 64 * ep[:, None])) % N) / N)
    L2[0, 0:32, 0::2] = T0.real
    L2[0, 64:96, 0::2] = T0.imag
    L2[0, 64, 0::2] = (-1.0) ** b
    L2[0, 32:64, 1::2] = T32.real
    L2[0, 96:128, 1::2] = T32.imag
    w0 = np.full(32, 2.0); w0[0] = 1.0
    L2i[0, :64, 0:32] = (T0.real * w0[:, None]).T
    L2i[0, :64, 64:96] = (T0.imag * w0[:, None]).T
    L2i[0, :64, 64] = (-1.0) ** b
    L2i[0, 64:, 32:64] = 2.0 * T32.real.T
    L2i[0, 64:, 96:128] = 2.0 * T32.imag.T
    S1i = np.zeros((32, 64))
    S1i[:, 0] = 1.0 / N
    S1i[:, 1] = ((-1.0) ** a) / N
    for c in range(1, 32):
        S1i[:, 2 * c] = 2 * np.cos(2 * np.pi * a * c / 64) / N
        S1i[:, 2 * c + 1] = -2 * np.sin(2 * np.pi * a * c / 64) / N
    LF = np.zeros((64, 128))
    for p in range(2):
        LF[p * 32:(p + 1) * 32, p * 64:(p + 1) * 64] = S1i
    return dict(L1h=L1h, L1k=L1k, L2=L2, L2i=L2i, LF=LF)


_M = make_consts()
_t = np.zeros_like(_M['L2i']); _t[:, :, 0::2] = _M['L2i'][:, :, :64]; _t[:, :, 1::2] = _M['L2i'][:, :, 64:]; _M['L2i'] = _t
def _group_rows(m):
    *lead, R2, C = m.shape
    R = R2 // 2
    m = m.reshape(*lead, 2, R // 8, 8, C)
    m = np.moveaxis(m, -4, -3)
    return m.reshape(*lead, R2, C)
_M = {k: _group_rows(v) for k, v in _M.items()}
def _gen_tables():
    k = np.arange(128); b = k // 2; odd = (k % 2 == 1)
    e = np.arange(8)
    F0 = np.exp(-2j * np.pi * ((e[:, None] * b[None, :]) % 64) / 64) * np.where(odd, 1j, 1.0)[None, :]
    w8 = np.exp(-2j * np.pi * (b % 8) / 8)
    s = np.arange(32)
    tw = np.exp(-2j * np.pi * (s[:, None] * b[None, :]) / 4096)
    g = np.zeros((176, 128))
    g[0:8] = F0.real; g[8:16] = F0.imag; g[16] = w8.real; g[17] = w8.imag
    g[24:56] = tw.real; g[56:88] = tw.imag
    col = np.arange(128); bi = 8 * (col // 16) + col % 8; cp = (col // 8) % 2
    row = np.arange(8); ee = row // 2; cc = row % 2
    phi = np.array([[1.0, -1j], [1j, 1.0]])[cp[None, :], cc[:, None]]
    G0 = np.exp(-2j * np.pi * ((ee[:, None] * bi[None, :]) % 64) / 64) * phi
    w4 = np.exp(-2j * np.pi * (bi % 16) / 16)
    twi = np.exp(-2j * np.pi * (s[:, None] * bi[None, :]) / 4096)
    g[88:96] = G0.real; g[96:104] = G0.imag; g[104] = w4.real; g[105] = w4.imag
    g[112:144] = twi.real; g[144:176] = twi.imag
    return g.astype(np.float32)
_GEN = _gen_tables()
_C = {k: pack_rows(np.ascontiguousarray(v)) for k, v in _M.items()}
def _const_blob():
    blob = np.zeros((128 + 32 + 176 + 128, 128), np.uint32)
    blob[0:64, 0:64] = _C['L1h']
    blob[64:128, 0:64] = _C['L1k']
    blob[128:160] = _C['LF']
    blob[160:336] = _GEN.view(np.uint32)
    blob[336:400] = _C['L2'][0]
    blob[400:464] = _C['L2i'][0]
    return blob
_BLOB = _const_blob()
KG = 16
KE = 32
ST1 = 36
ST2 = 68
STH = 68
STK = 36
OFF_Y = 0
PAD = 72
ZROWS = 32 * STK + PAD
T1ROWS = 64 * ST1 + PAD
OFF_Z = OFF_Y + 4096
OFF_Q = OFF_Z + 2 * ZROWS
OFF_G = OFF_Q + NB * 1024
AROWS = OFF_G + 2048 + PAD
NSTEP = NB

f32 = jnp.float32
bf16 = jnp.bfloat16
u32 = jnp.uint32


def _interleave(*lists):
    lists = [list(l) for l in lists if len(l)]
    items = []
    for li, l in enumerate(lists):
        for i, fn in enumerate(l):
            items.append(((i + 0.5) / len(l), li, i, fn))
    items.sort(key=lambda t: (t[0], t[1]))
    for _, _, _, fn in items:
        fn()


def _kernel(aw_hbm, bw_hbm, ad_hbm, bd_hbm, gw_hbm,
            q_hbm, ak_hbm, av_hbm, bk_hbm, bv_hbm, ah_hbm, bh_hbm, c_hbm,
            o_hbm,
            aw_ref, bw_ref, ad_ref, bd_ref, gw_ref, c_ref,
            hbuf, obuf, l2_ref, l2i_ref,
            hpA, hpB, kvA, kvB, t2A, t2B, arena, arena2, prm_ref,
            sem_k, sem_h, sem_q, sem_l, sem_o, sem_s, sem_t):
    j = pl.program_id(0)
    hp_ref = (hpA, hpB); kv_ref = (kvA, kvB);  t2_ref = (t2A, t2B)
    zero = jnp.minimum(j, 0)
    def aview(off, n, ar=arena):
        return ar.at[pl.ds(pl.multiple_of(zero + off, 8), n)]
    t1_ref = tuple(aview(8192 + i * T1ROWS, T1ROWS, arena2) for i in range(4))
    y_ref = (aview(OFF_Y, 2048), aview(OFF_Y + 2048, 2048))
    z_ref = (aview(OFF_Z, ZROWS), aview(OFF_Z + ZROWS, ZROWS))
    g_ref = aview(OFF_G, 2048 + PAD)
    l1h_w = lambda: pltpu.bitcast(c_ref[0:64, 0:64], bf16)
    l1k_w = lambda: pltpu.bitcast(c_ref[64:128, 0:64], bf16)
    lf_w = lambda: pltpu.bitcast(c_ref[128:160, :], bf16)
    def gen(r0, n):
        return pltpu.bitcast(c_ref[160 + r0:160 + r0 + n, :], f32)
    blk_of = lambda t: t
    jd = blk_of(j)
    jq = blk_of(jnp.maximum(j - 1, 0))
    slot = j % 2

    def unpack(x):
        e = pltpu.unpack_elementwise(x, index=0, packed_dtype=bf16, unpacked_dtype=f32)
        o = pltpu.unpack_elementwise(x, index=1, packed_dtype=bf16, unpacked_dtype=f32)
        return e, o

    def pack(lo, hi):
        return pltpu.pack_elementwise([lo, hi], packed_dtype=bf16)

    def asbf(x):
        return pltpu.bitcast(x, bf16)

    kv_hbm = (ak_hbm, av_hbm, bk_hbm, bv_hbm)
    h_hbm = (ah_hbm, bh_hbm)

    def cols(blk):
        return pl.ds(blk * 128, 128) if isinstance(blk, int) else pl.ds(pl.multiple_of(blk * 128, 128), 128)

    def kview(sl, i):
        return aview(sl * 4096 + i * 1024, 1024, arena2)

    def qview(blk):
        return aview(OFF_Q + blk * 1024, 1024)

    def k_copy(blk, sl, i):
        return pltpu.make_async_copy(kv_hbm[i].at[:, cols(blk)], kview(sl, i).bitcast(bf16), sem_k.at[sl, i])

    def h_copy(blk, sl, i):
        return pltpu.make_async_copy(h_hbm[i].at[cols(blk), :], hbuf.at[sl, i], sem_h.at[sl, i])

    def q_copy(i):
        return pltpu.make_async_copy(q_hbm.at[:, cols(i)], qview(i).bitcast(bf16), sem_q.at[i])

    def c_copy():
        return pltpu.make_async_copy(c_hbm, c_ref, sem_l.at[0])

    def o_copy(blk, sl):
        return pltpu.make_async_copy(obuf.at[sl], o_hbm.at[:, cols(blk)], sem_o.at[sl])

    def waits(*cs):
        def f():
            for c in cs:
                c.wait()
        return f

    row8 = jax.lax.broadcasted_iota(jnp.int32, (8, 128), 0)
    DD = lambda br: prm_ref[jd, pl.ds(8 + br, 1), :]

    def pk(r, g, c0=0):
        return pack(r[16 * g:16 * g + 8, c0:c0 + 128], r[16 * g + 8:16 * g + 16, c0:c0 + 128])

    def store_t1(ref, r, be, side=None, n0=0):
        for g in range(8):
            ref[pl.ds((2 * be + g // 4) * ST1 + 8 * (g % 4), 8), :] = pk(r, g)
            if side is not None:
                side(n0 + be * 8 + g)

    def hprep(br):
        def item(tau):
            def f():
                h_ref = hbuf.at[slot, br]
                x0 = h_ref[:, pl.ds(256 * tau, 128)].astype(f32)
                x1 = h_ref[:, pl.ds(256 * tau + 128, 128)].astype(f32)
                w = pack(x0, x1).T
                hp_ref[br][pl.ds((2 * tau) * STH, 64), :] = w[:64]
                hp_ref[br][pl.ds((2 * tau + 1) * STH, 64), :] = w[64:]
            return f
        return [item(t) for t in range(8)]

    def hstage(br, side=None, n0=0):
        def item(be):
            def f():
                x = jnp.concatenate([hp_ref[br][pl.ds(2 * be + p, 16, stride=STH), :] for p in range(2)], axis=0)
                r = jnp.dot(l1h_w(), asbf(x), preferred_element_type=f32)
                store_t1(t1_ref[2 * br], r, be, side, n0)
            return f
        return [item(be) for be in range(32)]

    def kprep(br, blk, sl):
        wc = []
        def item(m0):
            def f():
                if not wc:
                    wc.append(tuple(prm_ref[blk, pl.ds(4 * br + i, 1), :] for i in range(4)))
                w0, w1, w2, w3 = wc[0]
                ku = kview(sl, 2 * br)
                vu = kview(sl, 2 * br + 1)
                c = ku[pl.ds(m0, KG), :]
                if m0 == 0:
                    f8 = ku[pl.ds(0, 8), :]
                    p1 = jnp.where(row8 < 1, jnp.uint32(0), pltpu.roll(f8, 1, 0))
                    p2 = jnp.where(row8 < 2, jnp.uint32(0), pltpu.roll(f8, 2, 0))
                    if KG > 8:
                        p1 = jnp.concatenate([p1, ku[pl.ds(7, KG - 8), :]], axis=0)
                        p2 = jnp.concatenate([p2, ku[pl.ds(6, KG - 8), :]], axis=0)
                else:
                    p1 = ku[pl.ds(m0 - 1, KG), :]
                    p2 = ku[pl.ds(m0 - 2, KG), :]
                e, o = unpack(c)
                e1, o1 = unpack(p1)
                o2 = pltpu.unpack_elementwise(p2, index=1, packed_dtype=bf16, unpacked_dtype=f32)
                ve, vo = unpack(vu[pl.ds(m0, KG), :])
                kse = w0 * e + w1 * o1 + w2 * e1 + w3 * o2
                kso = w0 * o + w1 * e + w2 * o1 + w3 * e1
                kv_ref[br][pl.ds((m0 // 32) * STK + m0 % 32, KG), :] = pack(kse * ve, kso * vo)
            return f
        return [item(m0) for m0 in range(0, 1024, KG)]

    def kstage(br, side=None, n0=0):
        def item(be):
            def f():
                x = kv_ref[br][pl.ds(be, 32, stride=STK), :]
                r = jnp.dot(l1k_w(), asbf(x), preferred_element_type=f32)
                store_t1(t1_ref[2 * br + 1], r, be, side, n0)
            return f
        return [item(be) for be in range(32)]

    def s2(br, side=None):
        def item(s):
            def f():
                x = jnp.concatenate([t1_ref[2 * br + i][pl.ds(s, 64, stride=ST1), :] for i in range(2)], axis=1)
                zz = jnp.dot(asbf(l2_ref.at[s].bitcast(u32)[...]), asbf(x), preferred_element_type=f32)
                ddv = DD(br)
                for g in range(8):
                    gr = zz[16 * g:16 * g + 8, :128] + ddv
                    gi = zz[16 * g + 8:16 * g + 16, :128]
                    zr = zz[16 * g:16 * g + 8, 128:]
                    zi = zz[16 * g + 8:16 * g + 16, 128:]
                    if s == 0 and g == 0:
                        gi = jnp.where(row8 == 0, gi + ddv, gi)
                        yr = jnp.where(row8 == 0, zr * gr, zr * gr - zi * gi)
                        yi = jnp.where(row8 == 0, zi * gi, zr * gi + zi * gr)
                    else:
                        yr = zr * gr - zi * gi
                        yi = zr * gi + zi * gr
                    y_ref[br][pl.ds(s * 64 + 8 * g, 8), :] = pack(yr, yi)
                    if side is not None:
                        side(s * 8 + g)
            return f
        return [item(s) for s in range(32)]

    def paced(total, *lists, frac=1.0):
        pos = [0] * len(lists)
        def side(n):
            for li, l in enumerate(lists):
                due = min(len(l), int((n + 1) * len(l) / (total * frac)))
                while pos[li] < due:
                    l[pos[li]]()
                    pos[li] += 1
        return side

    def s2i(side=None):
        def item(s):
            def f():
                y = jnp.concatenate([y_ref[br][pl.ds(s * 64, 64), :] for br in range(2)], axis=1)
                u = jnp.dot(asbf(l2i_ref.at[s].bitcast(u32)[...]), asbf(y), preferred_element_type=f32)
                for g in range(8):
                    for br in range(2):
                        t2_ref[br][pl.ds(s * ST2 + 8 * g, 8), :] = pk(u, g, 128 * br)
                        if side is not None:
                            side(s * 16 + g * 2 + br)
            return f
        return [item(s) for s in range(32)]

    def fin():
        def item(be):
            def f():
                x = jnp.concatenate(
                    [jnp.concatenate([t2_ref[i][pl.ds(2 * be + p, 32, stride=ST2), :] for i in range(2)], axis=1)
                     for p in range(2)], axis=0)
                y = jnp.dot(lf_w(), asbf(x), preferred_element_type=f32)
                for g in range(4):
                    for br in range(2):
                        z_ref[br][pl.ds(8 * g * STK + be, 8, stride=STK), :] = pk(y, g, 128 * br)
            return f
        return [item(be) for be in range(32)]

    def epi(qoff, osl):
        def item(m0):
            def f():
                qu = aview(qoff, 1024)
                ou = obuf.at[osl].bitcast(u32)
                zrow = (m0 // 32) * STK + m0 % 32
                ae, ao = unpack(z_ref[0][pl.ds(zrow, KE), :])
                be_, bo = unpack(z_ref[1][pl.ds(zrow, KE), :])
                ge = pltpu.bitcast(g_ref[pl.ds(2 * m0, KE, stride=2), :], f32)
                go = pltpu.bitcast(g_ref[pl.ds(2 * m0 + 1, KE, stride=2), :], f32)
                qe, qo = unpack(qu[pl.ds(m0, KE), :])
                ou[pl.ds(m0, KE), :] = pack(qe * (be_ + ge * (ae - be_)), qo * (bo + go * (ao - bo)))
            return f
        return [item(m0) for m0 in range(0, 1024, KE)]

    def cmul(ar, ai, br_, bi_):
        return ar * br_ - ai * bi_, ar * bi_ + ai * br_

    def gen_fwd(slist):
        f0u, f0v = gen(0, 8), gen(8, 8)
        w8r, w8i = gen(16, 1), gen(17, 1)
        for s in slist:
            U, V = cmul(f0u, f0v, gen(24 + s, 1), gen(56 + s, 1))
            blocks = []
            for g in range(8):
                blocks += [U, V]
                if g < 7:
                    U, V = cmul(U, V, w8r, w8i)
            l2_ref[s] = jnp.concatenate(blocks, axis=0).astype(bf16)

    def gen_inv(slist):
        g0r, g0i = gen(88, 8), gen(96, 8)
        w4r, w4i = gen(104, 1), gen(105, 1)
        for s in slist:
            U, V = cmul(g0r, g0i, gen(112 + s, 1), gen(144 + s, 1))
            blocks = []
            for v in range(16):
                blocks.append(U)
                if v < 15:
                    U, V = cmul(U, V, w4r, w4i)
            l2i_ref[s] = jnp.concatenate(blocks, axis=0).T.astype(bf16)

    def gate():
        for i in range(NB):
            q_copy(i).wait()
        w = gw_ref[...].reshape(1, D)
        w16 = jnp.broadcast_to(w, (16, D))
        for c in range(4):
            qq = jnp.concatenate([asbf(qview(jb)[pl.ds(c * 256, 256), :]) for jb in range(NB)], axis=1)
            z = lax.dot_general(w16, qq, (((1,), (1,)), ((), ())), preferred_element_type=f32)
            g = 0.5 * jnp.tanh(0.5 * z[:8]) + 0.5
            for t in range(4):
                gt = jnp.broadcast_to(g[0:1, t * 128:(t + 1) * 128], (128, 128))
                g_ref[pl.ds((4 * c + t) * 128, 128), :] = pltpu.bitcast(gt.T, u32)

    osl = (j + 1) % 2

    def run(items):
        for it in items:
            it()

    small = ((aw_hbm, aw_ref), (bw_hbm, bw_ref), (ad_hbm, ad_ref), (bd_hbm, bd_ref), (gw_hbm, gw_ref))
    def s_copy(i):
        return pltpu.make_async_copy(small[i][0], small[i][1], sem_s.at[i])

    def start_k(blk, sl):
        for i in range(4):
            k_copy(blk, sl, i).start()

    def start_h(blk, sl):
        for i in range(2):
            h_copy(blk, sl, i).start()

    def wait_k(sl, idx=(0, 1, 2, 3)):
        for i in idx:
            k_copy(0, sl, i).wait()


    @pl.when(j == 0)
    def _first():
        c_copy().start()
        h_copy(0, 0, 0).start()
        g_ref[pl.ds(0, 2048), :] = jnp.zeros((2048, 128), u32)
        c_copy().wait()
        for i in range(len(small)):
            s_copy(i).start()
        k_copy(0, 0, 0).start()
        k_copy(0, 0, 1).start()
        l2_ref[0] = pltpu.bitcast(c_ref[336:400, :], bf16)
        l2i_ref[0] = pltpu.bitcast(c_ref[400:464, :], bf16)
        gen_fwd(range(1, 32))
        h_copy(0, 0, 0).wait()
        h_copy(0, 0, 1).start()
        run(hprep(0))
        _interleave(hstage(0), [lambda s=s: gen_inv([s]) for s in range(1, 20)])
        for i in range(len(small)):
            s_copy(i).wait()
        wait_k(0, (0, 1))
        k_copy(0, 0, 2).start()
        k_copy(0, 0, 3).start()
        adv = ad_ref[...].astype(f32).reshape(1, D)
        bdv = bd_ref[...].astype(f32).reshape(1, D)
        awv = aw_ref[...].astype(f32)
        bwv = bw_ref[...].astype(f32)
        for i in range(NB):
            c0 = i * 128
            prm_ref[i] = jnp.concatenate(
                [awv[:, c0:c0 + 128], bwv[:, c0:c0 + 128], adv[:, c0:c0 + 128], bdv[:, c0:c0 + 128],
                 jnp.zeros((6, 128), f32)], axis=0)
        run(kprep(0, 0, 0))
        h_copy(0, 0, 1).wait()
        start_k(1, 1)
        _interleave(kstage(0), hprep(1))
        gi = [lambda s=s: gen_inv([s]) for s in range(20, 32)]
        _interleave(s2(0), gi)
        wait_k(0, (2, 3))
        start_h(1, 1)
        run(hstage(1, paced(256, kprep(1, 0, 0))))
        run(kstage(1))
        run(s2(1))
        run(s2i())

    osl = (j + 1) % 2
    nxt = blk_of(jnp.minimum(j + 1, NSTEP - 1))

    @pl.when(j > 0)
    def _steady():
        more = j + 1 < NSTEP
        h_copy(0, slot, 0).wait()
        h_copy(0, slot, 1).wait()
        wait_k(slot)
        @pl.when(j == 1)
        def _():
            for i in range(NB):
                q_copy(i).start()
        @pl.when(more)
        def _():
            start_h(nxt, 1 - slot)
            start_k(nxt, 1 - slot)
        pl.when(j >= 3)(waits(o_copy(0, osl)))
        _interleave(fin(), hprep(0))
        kit = kprep(0, jd, slot) + kprep(1, jd, slot)
        n1, n2 = 28, 80
        _interleave(hstage(0, paced(256, kit[:n1]), 0) if n1 else hstage(0), hprep(1))
        run(hstage(1, paced(256, kit[n1:n2]), 0))
        run(kstage(0, paced(256, kit[n2:], frac=0.9), 0))
        run(kstage(1))
        ep = epi(jnp.where(j == 1, OFF_G, OFF_Q + jq * 1024), osl)
        run(s2(0, paced(256, ep[:len(ep) // 2])))
        run(s2(1, paced(256, ep[len(ep) // 2:])))
        run(s2i())
        @pl.when(j == 1)
        def _():
            gate()
            run(epi(OFF_Q + jq * 1024, osl))
        o_copy(jq, osl).start()

    @pl.when(j == NSTEP - 1)
    def _():
        osl2 = j % 2
        run(fin())
        o_copy(0, osl2).wait()
        ep2 = epi(OFF_Q + jd * 1024, osl2)
        NC = 8
        n = len(ep2) // NC
        cps = []
        for c in range(NC):
            run(ep2[c * n:(c + 1) * n])
            rows = pl.ds(c * (S // NC), S // NC)
            cp = pltpu.make_async_copy(obuf.at[osl2, rows, :], o_hbm.at[rows, cols(jd)], sem_t.at[c])
            cp.start()
            cps.append(cp)
        o_copy(0, osl).wait()
        for cp in cps:
            cp.wait()


@jax.jit
def pallas_gated_mix__ssm_conv_h3__ssm_conv_h3__prompt_kernel(A_q, A_k, A_v, A_shift_k, A_ssm_k, A_ssm_D, B_q, B_k, B_v, B_shift_k, B_ssm_k, B_ssm_D, gate_w):
    q = A_q.reshape(S, D)
    ak = A_k.reshape(S, D); av = A_v.reshape(S, D)
    bk = B_k.reshape(S, D); bv = B_v.reshape(S, D)
    aw = A_shift_k.T
    bw = B_shift_k.T
    vm = pl.BlockSpec(memory_space=pltpu.VMEM)
    anyspec = pl.BlockSpec(memory_space=pl.ANY)
    out = pl.pallas_call(
        _kernel,
        grid=(NSTEP,),
        in_specs=[anyspec] * 13,
        out_specs=anyspec,
        out_shape=jax.ShapeDtypeStruct((S, D), jnp.bfloat16),
        scratch_shapes=[
            pltpu.VMEM((4, D), bf16), pltpu.VMEM((4, D), bf16),
            pltpu.VMEM((D,), bf16), pltpu.VMEM((D,), bf16), pltpu.VMEM((D,), bf16),
            pltpu.VMEM(_BLOB.shape, u32),
            pltpu.VMEM((2, 2, 128, S), bf16),
            pltpu.VMEM((2, S, 128), bf16),
            pltpu.VMEM((32, 128, 128), bf16),
            pltpu.VMEM((32, 128, 128), bf16),
            *[pltpu.VMEM((16 * STH + PAD, 128), u32)] * 2,
            *[pltpu.VMEM((32 * STK + PAD, 128), u32)] * 2,
            *[pltpu.VMEM((32 * ST2 + PAD, 128), u32)] * 2,
            pltpu.VMEM((AROWS, 128), u32),
            pltpu.VMEM((8192 + 4 * T1ROWS, 128), u32),
            pltpu.VMEM((NB, 16, 128), f32),
            pltpu.SemaphoreType.DMA((2, 4)),
            pltpu.SemaphoreType.DMA((2, 2)),
            pltpu.SemaphoreType.DMA((NB,)),
            pltpu.SemaphoreType.DMA((1,)),
            pltpu.SemaphoreType.DMA((2,)),
            pltpu.SemaphoreType.DMA((5,)),
            pltpu.SemaphoreType.DMA((8,)),
        ],
        compiler_params=pltpu.CompilerParams(
            dimension_semantics=("arbitrary",), vmem_limit_bytes=100 * 1024 * 1024),
    )(aw, bw, A_ssm_D, B_ssm_D, gate_w,
      q, ak, av, bk, bv, A_ssm_k, B_ssm_k, jnp.asarray(_BLOB))
    return out.reshape(1, S, D)
```
